```python
import os as _os
_os.environ.setdefault("JAX_PLATFORMS", "cpu")
import jax
import jax.numpy as jnp

def _softmax(x, axis=-1):
    return jax.nn.softmax(x, axis=axis)
def _gelu(x):
    return jax.nn.gelu(x, approximate=True)
def _silu(x):
    return jax.nn.silu(x)
def _sigmoid(x):
    return jax.nn.sigmoid(x)
def _layernorm(x, axis=-1, eps=1e-5):
    m = jnp.mean(x, axis=axis, keepdims=True)
    v = jnp.var(x, axis=axis, keepdims=True)
    return (x - m) / jnp.sqrt(v + eps)
def _scatter_add(tgt, idx, src, axis=0):
    return tgt.at[idx].add(src)
def _segment_sum(src, seg, n):
    return jax.ops.segment_sum(src, seg, n)
class _Rng:
    def __init__(self, key):
        self._k = key
    def _next(self):
        self._k, sub = jax.random.split(self._k)
        return sub
    def normal(self, shape):
        return jax.random.normal(self._next(), shape, dtype=jnp.bfloat16)
    def randint(self, lo, hi, shape):
        return jax.random.randint(self._next(), shape, lo, hi, dtype=jnp.int32)
    def uniform(self, shape, lo=0.0, hi=1.0):
        return jax.random.uniform(self._next(), shape, jnp.bfloat16, lo, hi)
    def permutation(self, n):
        return jax.random.permutation(self._next(), n)


kernel_name = 'concat_heads__gqa_block_cached__mha_block_cached__near_ridge'

def setup_inputs():
    _rng = _Rng(jax.random.key(int.from_bytes(__import__("os").urandom(4), "little")))
    _w = (lambda a: (lambda t: t.astype(jnp.bfloat16) if jnp.issubdtype(t.dtype, jnp.floating) else t)(jnp.asarray(a)))
    def _A_setup():
        B, Sq, D = 8, 96, 640
        Hq, Hkv, Sk, Dh = 32, 32, 512, 128
        assert Hq % Hkv == 0, (Hq, Hkv)
        return {
            "x": _w((lambda *s: _rng.normal(s) * 0.8)(B, Sq, D)),
            "k_cache": _w((lambda *s: _rng.normal(s) * 0.8)(B, Hkv, Sk, Dh)),
            "v_cache": _w((lambda *s: _rng.normal(s) * 0.05)(B, Hkv, Sk, Dh)),
            "wq": _w((lambda *s: _rng.normal(s) * 0.8)(D, Hq * Dh) * (D ** -0.5)),
            "wo": _w((lambda *s: _rng.normal(s) * 0.05)(Hq * Dh, D) * ((Hq * Dh) ** -0.5)),
        }
    _A_in = _A_setup()

    def _B_setup():
        B, Sq, D = 8, 96, 640
        H, Sk, Dh = 32, 512, 128
        return {
            "x": _w((lambda *s: _rng.normal(s) * 0.8)(B, Sq, D)),
            "k_cache": _w((lambda *s: _rng.normal(s) * 0.8)(B, H, Sk, Dh)),
            "v_cache": _w((lambda *s: _rng.normal(s) * 0.05)(B, H, Sk, Dh)),
            "wq": _w((lambda *s: _rng.normal(s) * 0.8)(D, H * Dh) * (D ** -0.5)),
            "wo": _w((lambda *s: _rng.normal(s) * 0.05)(H * Dh, D) * ((H * Dh) ** -0.5)),
        }
    _B_in = _B_setup()

    return {
        "A_x": _A_in["x"],
        "A_k_cache": _A_in["k_cache"],
        "A_v_cache": _A_in["v_cache"],
        "A_wq": _A_in["wq"],
        "A_wo": _A_in["wo"],
        "B_x": _B_in["x"],
        "B_k_cache": _B_in["k_cache"],
        "B_v_cache": _B_in["v_cache"],
        "B_wq": _B_in["wq"],
        "B_wo": _B_in["wo"],
    }

def reference(A_x, A_k_cache, A_v_cache, A_wq, A_wo, B_x, B_k_cache, B_v_cache, B_wq, B_wo):
    def _A_ref(x, k_cache, v_cache, wq, wo):
        B, Sq, D = x.shape
        Hq, Dh = 32, 128
        Hkv = k_cache.shape[1]
        rep = Hq // Hkv
        q = (lambda x, *d: x.transpose(*d))((x @ wq).reshape(B, Sq, Hq, Dh), 0, 2, 1, 3)
        k = jnp.repeat(k_cache, rep, axis=1)
        v = jnp.repeat(v_cache, rep, axis=1)
        scores = jnp.einsum("bhqd,bhkd->bhqk", q, k) * (Dh ** -0.5)
        p = _softmax(scores, axis=-1)
        o = jnp.einsum("bhqk,bhkd->bhqd", p, v)
        return (lambda x, *d: x.transpose(*d))(o, 0, 2, 1, 3).reshape(B, Sq, Hq * Dh) @ wo

    def _B_ref(x, k_cache, v_cache, wq, wo):
        B, Sq, D = x.shape
        H, Dh = 32, 128
        q = (lambda x, *d: x.transpose(*d))((x @ wq).reshape(B, Sq, H, Dh), 0, 2, 1, 3)
        scores = jnp.einsum("bhqd,bhkd->bhqk", q, k_cache) * (Dh ** -0.5)
        p = _softmax(scores, axis=-1)
        o = jnp.einsum("bhqk,bhkd->bhqd", p, v_cache)
        return (lambda x, *d: x.transpose(*d))(o, 0, 2, 1, 3).reshape(B, Sq, H * Dh) @ wo

    a = _A_ref(A_x, A_k_cache, A_v_cache, A_wq, A_wo)
    b = _B_ref(B_x, B_k_cache, B_v_cache, B_wq, B_wo)
    return jnp.concatenate([a, b], axis=-1)
```

```python
import jax, jax.numpy as jnp
import jax.experimental.pallas as pl
import jax.experimental.pallas.tpu as pltpu

B, SQ, D, H, SK, DH = 8, 96, 640, 32, 512, 128
M = B * SQ
QSCALE = float(DH ** -0.5 * 1.4426950408889634)
BF, F32 = jnp.bfloat16, jnp.float32

def make(wqm=(128, 128), wom=(64, 640), xm=(128, 128), oa=(128, 128), obm=(96, 128), wpos='front', lag=1, compute=True,
         flags=None, kvo='tsb', nis=8, halves=1, na=8, view=0, pro_loop=False, dist=16, flip=0, a0=0):
    NS = 3 if dist <= 16 else 4; NG = 2 * H
    def kern(ax, ak, av, awq, awo, bx, bk, bv, bwq, bwo, out, kb, vb, wqb, wob, xb, qb, ob, acc, stage, sems, xsem, osem):
        A, Bq = (ak, av, awq, awo), (bk, bv, bwq, bwo)
        def tiles(r0, nr, c0, nc, shp):
            return [(pl.ds(r0 + i, shp[0]), pl.ds(c0 + j, shp[1])) for j in range(0, nc, shp[1]) for i in range(0, nr, shp[0])]
        def packet(refs, h, s):
            k, v, wq, wo = refs
            hq = pl.multiple_of(h * DH, DH)
            w = [(wq.at[r, pl.ds(hq, DH)], wqb.at[s, r], sems.at[s]) for r, _ in tiles(0, D, 0, DH, wqm)]
            if view: w += [(wo.at[h * 5 + j], wob.at[s, :, pl.ds(j * 128, 128)], sems.at[s]) for j in range(5)]
            else: w += [(wo.at[pl.ds(hq + r.start, r.size), c], wob.at[s, r, c], sems.at[s]) for r, c in tiles(0, DH, 0, D, wom)]
            n = B // halves
            mk = lambda t, b, j: ((k, v)[t].at[b, h, pl.ds(j * 128, 128)], (kb, vb)[t].at[s, b, pl.ds(j * 128, 128)], sems.at[(b // n) * NS + s])
            if kvo == 'tsb': kv = [mk(t, p * n + b, j) for p in range(halves) for t in (0, 1) for j in range(4) for b in range(n)]
            elif kvo == 'stb': kv = [mk(t, p * n + b, j) for p in range(halves) for j in range(4) for t in (0, 1) for b in range(n)]
            elif kvo == 'sbt': kv = [mk(t, p * n + b, j) for p in range(halves) for j in range(4) for b in range(n) for t in (0, 1)]
            if wpos == 'mid': return kv[:32] + w + kv[32:]
            if wpos == 'mix':
                res = []
                for i in range(8): res += w[2 * i:2 * i + 2] + kv[8 * i:8 * i + 8]
                return res + w[16:]
            return w + kv
        def start(cs, lo=0, hi=None):
            for n, c in list(enumerate(cs))[lo:hi]: pltpu.make_async_copy(*c).start(priority=(n + flip) % 2)
        def wait_all(ref, sem): pltpu.make_async_copy(ref, ref, sem).wait()
        def issue(g, t):
            for i, refs in enumerate((A, Bq)):
                @pl.when(g // H == i)
                def _():
                    cs = packet(refs, g % H, g % NS)
                    start(cs, len(cs) * t // nis, len(cs) * (t + 1) // nis)
        xcp = lambda i: [((ax, bx)[i].at[t], xb.at[i].at[t], xsem) for t in tiles(0, M, 0, D, xm)]
        start(xcp(0) + xcp(1))
        acc[...] = jnp.zeros(acc.shape, F32)
        nfull, rem = divmod(dist * nis // 8, nis)
        if pro_loop: jax.lax.fori_loop(0, nfull, lambda g, _: start(packet(A, g, g)), None)
        else:
            for g in range(nfull): start(packet(A, g, g))
        cs = packet(A, nfull, nfull); start(cs, 0, len(cs) * rem // nis)
        wait_all(xb, xsem)
        rows = lambda b: pl.ds(b * SQ, SQ)
        def step(g, _):
            s = g % NS; br = g // H; n = B // halves
            sc = {}
            for t in range(B + lag + 2):
                if t == 0:
                    wait_all(wqb.at[s], sems.at[s]); wait_all(wob.at[s], sems.at[s])
                    for buf in (kb, vb): wait_all(buf.at[s, pl.ds(0, n)], sems.at[s])
                if t < nis: issue(g + nfull + (t + rem) // nis, (t + rem) % nis)
                if a0 <= t < a0 + na:
                    @pl.when(g == NG - 1)
                    def _():
                        oc = [(stage.at[0, r, c], out.at[r, c], osem) for r, c in tiles(0, M, 0, D, oa)]
                        start(oc, len(oc) * (t - a0) // na, len(oc) * (t - a0 + 1) // na)
                if t < B and compute:
                    q = jnp.dot(xb[br, rows(t), :], wqb[s], preferred_element_type=F32)
                    qb[rows(t), :] = (q * QSCALE).astype(BF)
                b = t - 1
                if 0 <= b < B:
                    if b > 0 and b % n == 0:
                        for buf in (kb, vb): wait_all(buf.at[s, pl.ds(b, n)], sems.at[(b // n) * NS + s])
                    if compute: sc[b] = jax.lax.dot_general(qb[rows(b), :], kb[s, b], (((1,), (1,)), ((), ())), preferred_element_type=F32)
                b = t - 1 - lag
                if 0 <= b < B and compute:
                    x = sc.pop(b)
                    p = jnp.exp2(x - jnp.max(x, axis=-1, keepdims=True))
                    l = jnp.sum(p, axis=-1, keepdims=True)
                    o = jnp.dot(p.astype(BF), vb[s, b], preferred_element_type=F32)
                    ob[rows(b), :] = (o * (1.0 / l)).astype(BF)
                b = t - 2 - lag
                if 0 <= b < B:
                    if compute:
                        r = acc[br, rows(b), :] + jnp.dot(ob[rows(b), :], wob[s], preferred_element_type=F32)
                        acc[br, rows(b), :] = r
                        stage[br, rows(b), :] = r.astype(BF)
                    @pl.when(g == NG - 1)
                    def _(): start([(stage.at[1, r_, c], out.at[r_, pl.ds(D + c.start, c.size)], osem) for r_, c in tiles(b * SQ, SQ, 0, D, obm)])
        jax.lax.fori_loop(0, NG, step, None)
        wait_all(stage, osem)
    @jax.jit
    def f(ax, ak, av, awq, awo, bx, bk, bv, bwq, bwo):
        if view: awo, bwo = [w.reshape(512, 8, 5, 128).transpose(0, 2, 1, 3).reshape(160, 128, 128) for w in (awo, bwo)]
        o = pl.pallas_call(kern, out_shape=jax.ShapeDtypeStruct((M, 2 * D), BF),
            in_specs=[pl.BlockSpec(memory_space=pltpu.HBM)] * 10, out_specs=pl.BlockSpec(memory_space=pltpu.HBM),
            scratch_shapes=[pltpu.VMEM((NS, B, SK, DH), BF), pltpu.VMEM((NS, B, SK, DH), BF), pltpu.VMEM((NS, D, DH), BF), pltpu.VMEM((NS, DH, D), BF),
                pltpu.VMEM((2, M, D), BF), pltpu.VMEM((M, DH), BF), pltpu.VMEM((M, DH), BF), pltpu.VMEM((2, M, D), F32), pltpu.VMEM((2, M, D), BF),
                pltpu.SemaphoreType.DMA((NS * halves,)), pltpu.SemaphoreType.DMA(()), pltpu.SemaphoreType.DMA(())],
            compiler_params=pltpu.CompilerParams(vmem_limit_bytes=100 * 2**20, disable_bounds_checks=True, flags=flags), name="attn2",
        )(ax.reshape(M, D), ak, av, awq, awo, bx.reshape(M, D), bk, bv, bwq, bwo)
        return o.reshape(B, SQ, 2 * D)
    return f


@jax.jit
def pallas_concat_heads__gqa_block_cached__mha_block_cached__near_ridge_kernel(
        A_x, A_k_cache, A_v_cache, A_wq, A_wo, B_x, B_k_cache, B_v_cache, B_wq, B_wo):
    return make(halves=2, kvo='stb', dist=12)(A_x, A_k_cache, A_v_cache, A_wq, A_wo, B_x, B_k_cache, B_v_cache, B_wq, B_wo)
```

```python
import jax, jax.numpy as jnp
import jax.experimental.pallas as pl
import jax.experimental.pallas.tpu as pltpu

B, SQ, D, H, SK, DH = 8, 96, 640, 32, 512, 128
M = B * SQ
QSCALE = float(DH ** -0.5 * 1.4426950408889634)
BF, F32 = jnp.bfloat16, jnp.float32
NT = D // 128

def make(oa=(128, 128), obm=(96, 128), lag=1, compute=True, flags=None, a0=0, na=4, d=(12, 20), od=('s', 's'), wsw=0, wr=1, split=1, dyn=0,
         seq='dsqpo', olag=1, op=None, wt=0, first=0, pre=0):
    NS = 4; NG = 2 * H; GQ = 16; HB = B // 2
    def kern(ax, ak, av, awq, awo, bx, bk, bv, bwq, bwo, out, kb, vb, wqb, wop, wob, xp, xb, qb, ob, acc, stage, sems, qsem, xsem, osem):
        def tiles(r0, nr, c0, nc, shp):
            return [(pl.ds(r0 + i, shp[0]), pl.ds(c0 + j, shp[1])) for j in range(0, nc, shp[1]) for i in range(0, nr, shp[0])]
        def wq_page(wq, half, slot, part, e):
            r = pl.ds(pl.multiple_of(part * 8 + e * GQ * 8, 8), 8)
            return (wq.at[r, pl.ds(pl.multiple_of(half * 2048, 2048), 2048)], wqb.at[slot, r], qsem.at[slot])
        def go(c, n): pltpu.make_async_copy(*c).start(priority=n % 2)
        def start(cs, lo=0, hi=None, p=None):
            for n, c in list(enumerate(cs))[lo:hi]: go(c, n if p is None else p)
        def wait_all(ref, sem): pltpu.make_async_copy(ref, ref, sem).wait()
        def scal(g):
            gq = g + 1; grp = (gq >> 4) + 1; s = g & (NS - 1)
            return dict(h=g & (H - 1), s=s, s2=jnp.where(g == NG - 1, NS, s) if split else s, half=grp & 1, slot=grp & 3, part=gq & (GQ - 1), last=g == NG - 1,
                        kv=(g < H, (g >= H) & (g < NG)), wq=(gq < GQ, (gq >= GQ) & (gq < H + GQ)))
        def lst(th, o):
            if o == 's': return [(a, 2 * b + th, j) for j in range(4) for a in (0, 1) for b in range(HB)]
            if o == 'r': return [(a, 2 * b + 1 - th, j) for j in range(4) for a in (0, 1) for b in range(HB)]
            if o == 'x': return [(a, 2 * b + (th ^ a), j) for j in range(4) for a in (0, 1) for b in range(HB)]
            if o == 'h': return [(a, 4 * p + 2 * b + th, 2 * jj + j) for p in (0, 1) for jj in (0, 1) for a in (0, 1) for j in (0, 1) for b in (0, 1)]
            if o == 'g': return [(a, 4 * p + 2 * b + th, j) for p in (0, 1) for j in range(4) for a in (0, 1) for b in (0, 1)]
        def issue(cs, only_a=False):
            when = (lambda p: (lambda f: f())) if only_a else pl.when
            srcs = ((ak, av, awo, awq), (bk, bv, bwo, bwq))[:1 if only_a else 2]
            for e in range(-1, 4):
                for th in ((0, 1), (1, 0))[first]:
                    if cs[th] is None: continue
                    c, t = cs[th]; h, s = c['h'], c['s']; tw = t - wt
                    for i, (k, v, wo, wq) in enumerate(srcs):
                        if e >= 0:
                            a, b, j = lst(th, od[th])[4 * t + e]; sm = c['s2'] if b >= HB else s
                            if dyn and th == 1 and i == 1:
                                a2, b2, j2 = lst(th, 'h')[4 * t + e]; assert a2 == a
                                b, j = [x if x == y else jnp.where(c['last'], y, x) for x, y in ((b, b2), (j, j2))]
                                sm = c['s2'] if b2 >= HB else s
                            r = pl.ds(j * 128 if isinstance(j, int) else pl.multiple_of(j * 128, 128), 128)
                            when(c['kv'][i])(lambda: go(((k, v)[a].at[b, h, r], (kb, vb)[a].at[s, b, r], sems.at[sm]), th))
                        elif 0 <= tw < NT and th == wsw: when(c['kv'][i])(lambda: go((wo.at[h * NT + tw], wop.at[s, pl.ds(tw * 128, 128)], sems.at[s]), th))
                        elif 0 <= tw < NT: when(c['wq'][i])(lambda: go(wq_page(wq, c['half'], c['slot'], c['part'], tw), th))
        def unpage(w, n):
            w = w.astype(F32)
            return jnp.concatenate([jnp.concatenate([w[(r * NT + j) * 8:(r * NT + j + 1) * 8] for r in range(n)], axis=0) for j in range(NT)], axis=1).astype(BF)
        rows = lambda b: pl.ds(b * SQ, SQ)
        def qproj(g, r):
            q = jnp.dot(xb[g >> 5, r, :], wqb[g >> 4, :, pl.ds(pl.multiple_of((g & (GQ - 1)) * DH, DH), DH)], preferred_element_type=F32)
            qb[r, :] = (q * QSCALE).astype(BF)
        start([((ax, bx)[i].at[(p * 7) % 30], xp.at[i, pl.ds((p * 7) % 30 * 128, 128)], xsem) for p in range(30) for i in (0, 1)])
        jax.lax.fori_loop(0, GQ // 2, lambda p, _: start([wq_page(awq, 0, 0, p + i * GQ // 2, e) for i in (0, 1) for e in range(NT)]), None)
        start([wq_page(awq, 1, 1, 0, e) for e in range(NT)])
        for u in range(-max(d), 0): issue([(scal((u + x) // 8), (u + x) % 8) if u + x >= 0 else None for x in d], True)
        wait_all(xp, xsem); wait_all(wqb.at[0], qsem.at[0])
        def init(i, _):
            r = pl.ds(pl.multiple_of(i * 128, 128), 128)
            for j in range(2):
                acc[j, r, :] = jnp.zeros((128, D), F32)
                xb[j, r, :] = unpage(xp[j, pl.ds(pl.multiple_of(i * D, D), D), :], 16)
            qproj(0, r)
        jax.lax.fori_loop(0, M // 128, init, None)
        def step(g, fin):
            s = g & (NS - 1); br = g >> 5
            if not fin:
                cc = {i: scal(g + i) for i in range(min(d) // 8, (max(d) + 7) // 8 + 1)}
                pl.when((g + 1) & (GQ - 1) == 0)(lambda: wait_all(wqb.at[(g + 1) >> 4], qsem.at[(g + 1) >> 4]))
                @pl.when(g == H + 8)
                def _(): stage[:, pl.ds(0, D)] = acc[0].astype(BF)
            oc = [(stage.at[t_], out.at[t_], osem) for t_ in tiles(0, M, 0, D, oa)]
            if fin and wr: start(oc, 0, pre, op)
            wait_all(wop.at[s], sems.at[s])
            for buf in (kb, vb): wait_all(buf.at[s, pl.ds(0, HB)] if fin and split else buf.at[s], sems.at[s])
            if compute: wob[...] = unpage(wop[s], 16)
            sc = {}
            for t in range(B + lag + olag):
                for ph in seq:
                    if ph == 'd' and not fin and t < B: issue([(cc[(t + x) // 8], (t + x) % 8) for x in d])
                    if ph == 'd' and fin:
                        if t == HB and split:
                            for buf in (kb, vb): wait_all(buf.at[s, pl.ds(HB, HB)], sems.at[NS])
                        if a0 <= t < a0 + na and wr:
                            start(oc, pre + (len(oc) - pre) * (t - a0) // na, pre + (len(oc) - pre) * (t - a0 + 1) // na, op)
                    if ph == 's' and t < B and compute: sc[t] = jax.lax.dot_general(qb[rows(t), :], kb[s, t], (((1,), (1,)), ((), ())), preferred_element_type=F32)
                    if ph == 'q' and t < B and compute and not fin: qproj(g + 1, rows(t))
                    b = t - lag
                    if ph == 'p' and 0 <= b < B and compute:
                        x = sc.pop(b)
                        p = jnp.exp2(x - jnp.max(x, axis=-1, keepdims=True))
                        l = jnp.sum(p, axis=-1, keepdims=True)
                        o = jnp.dot(p.astype(BF), vb[s, b], preferred_element_type=F32)
                        ob[rows(b), :] = (o * (1.0 / l)).astype(BF)
                    b = t - lag - olag
                    if ph == 'o' and 0 <= b < B:
                        if compute:
                            r = acc[br, rows(b), :] + jnp.dot(ob[rows(b), :], wob[...], preferred_element_type=F32)
                            if fin: stage[rows(b), pl.ds(D, D)] = r.astype(BF)
                            else: acc[br, rows(b), :] = r
                        if fin and wr: start([(stage.at[t_], out.at[t_], osem) for t_ in tiles(b * SQ, SQ, D, D, obm)], p=op)
        jax.lax.fori_loop(0, NG - 1, lambda g, _: step(g, False), None)
        step(NG - 1, True)
        if wr: wait_all(stage, osem)
    @jax.jit
    def f(ax, ak, av, awq, awo, bx, bk, bv, bwq, bwo):
        pg = lambda w: w.reshape(-1, 8, NT, 128).transpose(0, 2, 1, 3).reshape(-1, 128, 128)
        o = pl.pallas_call(kern, out_shape=jax.ShapeDtypeStruct((M, 2 * D), BF),
            in_specs=[pl.BlockSpec(memory_space=pltpu.HBM)] * 10, out_specs=pl.BlockSpec(memory_space=pltpu.HBM),
            scratch_shapes=[pltpu.VMEM((NS, B, SK, DH), BF), pltpu.VMEM((NS, B, SK, DH), BF), pltpu.VMEM((4, D, 2048), BF), pltpu.VMEM((NS, D, DH), BF), pltpu.VMEM((DH, D), BF),
                pltpu.VMEM((2, M * NT, 128), BF), pltpu.VMEM((2, M, D), BF), pltpu.VMEM((M, DH), BF), pltpu.VMEM((M, DH), BF), pltpu.VMEM((2, M, D), F32), pltpu.VMEM((M, 2 * D), BF),
                pltpu.SemaphoreType.DMA((NS + 1,)), pltpu.SemaphoreType.DMA((4,)), pltpu.SemaphoreType.DMA(()), pltpu.SemaphoreType.DMA(())],
            compiler_params=pltpu.CompilerParams(vmem_limit_bytes=100 * 2**20, disable_bounds_checks=True, flags=flags), name="attn2",
        )(pg(ax), ak, av, awq, pg(awo), pg(bx), bk, bv, bwq, pg(bwo))
        return o.reshape(B, SQ, 2 * D)
    return f


@jax.jit
def pallas_concat_heads__gqa_block_cached__mha_block_cached__near_ridge_kernel(
        A_x, A_k_cache, A_v_cache, A_wq, A_wo, B_x, B_k_cache, B_v_cache, B_wq, B_wo):
    return make(split=0,pre=30)(A_x, A_k_cache, A_v_cache, A_wq, A_wo, B_x, B_k_cache, B_v_cache, B_wq, B_wo)
```

```python
import jax
import jax.numpy as jnp
import jax.experimental.pallas as pl
import jax.experimental.pallas.tpu as pltpu

B, SQ, D, H, SK, DH = 8, 96, 640, 32, 512, 128
M = B * SQ
STEPS = 2 * H
HALF = B // 2
LANES, TILE_ROWS = 128, 8
PAGE = 128
NT = D // LANES
X_PAGES = M * NT // PAGE
WQ_HEADS = 16
WQ_COLS = WQ_HEADS * DH
SLOTS = 4
Q_AHEAD = 3
AHEAD = (12, 20)
OUT_ROWS = 32
Q_SCALE = DH ** -0.5 * 1.4426950408889634


def _kv_pages(queue, by_halves):
    if by_halves:
        return [(a, HALF * p + 2 * b + queue, 2 * jj + j) for p in range(2) for jj in range(2)
                for a in range(2) for j in range(2) for b in range(2)]
    return [(a, 2 * b + queue, j) for j in range(SK // PAGE) for a in range(2) for b in range(HALF)]


def _block(i, size):
    return pl.ds(i * size if isinstance(i, int) else pl.multiple_of(i * size, size), size)


def _untile(pages):
    w = pages.astype(jnp.float32)
    tile = lambda r, c: w[(r * NT + c) * TILE_ROWS:(r * NT + c + 1) * TILE_ROWS]
    cols = [jnp.concatenate([tile(r, c) for r in range(128 // TILE_ROWS)], axis=0) for c in range(NT)]
    return jnp.concatenate(cols, axis=1).astype(pages.dtype)


def _attention_kernel(
        ax, ak, av, awq, awo, bx, bk, bv, bwq, bwo, out,
        k_buf, v_buf, wq_buf, wo_pages, wo_buf, x_pages, x_buf, q_buf, o_buf, acc, out_buf,
        k_sem, v_sem, wq_sem, wo_sem, x_sem, out_sem):
    blocks = ((ak, av, awq, awo), (bk, bv, bwq, bwo))

    def start(src, dst, sem, queue):
        pltpu.make_async_copy(src, dst, sem).start(priority=queue)

    def wait_filled(buf, sem):
        pltpu.make_async_copy(buf, buf, sem).wait()

    def start_wq_page(wq, group, part, e, queue):
        rows = _block(part + e * WQ_HEADS, TILE_ROWS)
        start(wq.at[rows, _block(group & 1, WQ_COLS)], wq_buf.at[group, rows], wq_sem.at[group], queue)

    def plan(g):
        slot = g & (SLOTS - 1)
        gq = g + Q_AHEAD
        return dict(
            head=g & (H - 1), slot=slot, last=g == STEPS - 1,
            late_sem=jnp.where(g >= STEPS - Q_AHEAD, SLOTS + slot, slot),
            wq_group=((gq >> 4) + 1) & 3, wq_part=gq & (WQ_HEADS - 1),
            kv_from=(g < H, (g >= H) & (g < STEPS)),
            wq_from=(gq < WQ_HEADS, (gq >= WQ_HEADS) & (gq < H + WQ_HEADS)))

    def prefetch(work, sources=(0, 1), with_wq=True):
        for e in range(-1, 4):
            for queue, item in enumerate(work):
                if item is None:
                    continue
                p, part = item
                for i in sources:
                    k, v, wq, wo = blocks[i]
                    if e >= 0:
                        a, b, j = _kv_pages(queue, False)[4 * part + e]
                        late = b >= HALF
                        sem = p["late_sem"] if late else p["slot"]
                        if queue == 1 and i == 1:
                            _, b2, j2 = _kv_pages(queue, True)[4 * part + e]
                            sem2 = p["late_sem"] if b2 >= HALF else p["slot"]
                            if late != (b2 >= HALF):
                                sem = jnp.where(p["last"], sem2, sem)
                            b = b if b == b2 else jnp.where(p["last"], b2, b)
                            j = j if j == j2 else jnp.where(p["last"], j2, j)
                        pl.when(p["kv_from"][i])(lambda: start(
                            (k, v)[a].at[b, p["head"], _block(j, PAGE)],
                            (k_buf, v_buf)[a].at[p["slot"], b, _block(j, PAGE)],
                            (k_sem, v_sem)[a].at[sem], queue))
                    elif part < NT and queue == 0:
                        pl.when(p["kv_from"][i])(lambda: start(
                            wo.at[p["head"] * NT + part], wo_pages.at[p["slot"], _block(part, PAGE)],
                            wo_sem.at[p["slot"]], queue))
                    elif part < NT and with_wq:
                        pl.when(p["wq_from"][i])(lambda: start_wq_page(
                            wq, p["wq_group"], p["wq_part"], part, queue))

    def project_q(g, rows):
        w = wq_buf[g >> 4, :, _block(g & (WQ_HEADS - 1), DH)]
        q = jnp.dot(x_buf[g >> 5, rows, :], w, preferred_element_type=jnp.float32)
        q_buf[g & (SLOTS - 1), rows, :] = (q * Q_SCALE).astype(q_buf.dtype)

    def start_output(i, r, queue):
        rows = _block(r, OUT_ROWS)
        start(out_buf.at[i, rows], out.at[rows, _block(i, D)], out_sem, queue)

    def first_pages(i, _):
        for e in range(NT):
            start_wq_page(awq, 0, i, e, e % 2)
        for j in range(4):
            page = i + (X_PAGES // 2) * (j // 2)
            pl.when(i < X_PAGES // 2)(lambda: start(
                (ax, bx)[j % 2].at[page], x_pages.at[j % 2, _block(page, PAGE)], x_sem, (j + 1) % 2))
        for j in range(Q_AHEAD):
            pl.when(i < NT)(lambda: start_wq_page(awq, 1, j, i, (j + 1) % 2))

    def run_ahead(lo, hi):
        for u in range(lo, hi):
            prefetch([(plan((u + d) // B), (u + d) % B) if u + d >= 0 else None for d in AHEAD], sources=(0,))

    def clear_acc(i, _):
        for j in range(2):
            acc[j, _block(i, 128), :] = jnp.zeros((128, D), acc.dtype)

    def untile_x(i, _):
        for j in range(2):
            x_buf[j, _block(i, 128), :] = _untile(x_pages[j, _block(i, NT * 128), :])

    jax.lax.fori_loop(0, WQ_HEADS, first_pages, None)
    jax.lax.fori_loop(0, M // 128, clear_acc, None)
    run_ahead(-max(AHEAD), -2 * Q_AHEAD)
    wait_filled(x_pages, x_sem)
    wait_filled(wq_buf.at[0], wq_sem.at[0])
    jax.lax.fori_loop(0, M // 128, untile_x, None)
    for g in range(Q_AHEAD):
        run_ahead(-2 * (Q_AHEAD - g), -2 * (Q_AHEAD - g - 1))
        jax.lax.fori_loop(0, 2, lambda i, _: project_q(g, _block(i, M // 2)), None)

    def step(g, tail):
        slot, blk = g & (SLOTS - 1), g >> 5
        plans = {i: plan(g + i) for i in range(min(AHEAD) // B, (max(AHEAD) + B - 1) // B + 1)}
        when_last = pl.when(g == STEPS - 1)
        if tail:
            for buf, sem in ((k_buf, k_sem), (v_buf, v_sem)):
                wait_filled(buf.at[slot, pl.ds(0, HALF)], sem.at[slot])
        else:
            group = (g + Q_AHEAD) >> 4
            pl.when(((g + Q_AHEAD) & (WQ_HEADS - 1)) == 0)(
                lambda: wait_filled(wq_buf.at[group], wq_sem.at[group]))

            @pl.when(g == H + B)
            def _():
                out_buf[0] = acc[0].astype(out_buf.dtype)

            for buf, sem in ((k_buf, k_sem), (v_buf, v_sem)):
                wait_filled(buf.at[slot], sem.at[slot])
        wait_filled(wo_pages.at[slot], wo_sem.at[slot])
        wo_buf[...] = _untile(wo_pages[slot])

        scores = {}
        for t in range(B + 2):
            if t < B:
                work = [(plans[(t + d) // B], (t + d) % B) if not tail or (t + d) // B < Q_AHEAD else None
                        for d in AHEAD]
                prefetch(work, sources=(1,) if tail else (0, 1), with_wq=not tail)
            if tail and t == 1:
                @when_last
                def _():
                    n = M // OUT_ROWS
                    for i in range(n):
                        start_output(0, (7 * i) % n, i % 2)
            if tail and t == HALF:
                for buf, sem in ((k_buf, k_sem), (v_buf, v_sem)):
                    wait_filled(buf.at[slot, pl.ds(HALF, HALF)], sem.at[SLOTS + slot])
            if t < B:
                scores[t] = jax.lax.dot_general(
                    q_buf[slot, _block(t, SQ), :], k_buf[slot, t], (((1,), (1,)), ((), ())),
                    preferred_element_type=jnp.float32)
                if not tail:
                    project_q(g + Q_AHEAD, _block(t, SQ))
            b = t - 1
            if 0 <= b < B:
                s = scores.pop(b)
                p = jnp.exp2(s - jnp.max(s, axis=-1, keepdims=True))
                total = jnp.sum(p, axis=-1, keepdims=True)
                o = jnp.dot(p.astype(v_buf.dtype), v_buf[slot, b], preferred_element_type=jnp.float32)
                o_buf[_block(b, SQ), :] = (o * (1.0 / total)).astype(o_buf.dtype)
            b = t - 2
            if 0 <= b < B:
                rows = _block(b, SQ)
                y = acc[blk, rows, :] + jnp.dot(o_buf[rows, :], wo_buf[...], preferred_element_type=jnp.float32)
                acc[blk, rows, :] = y
                if tail:
                    out_buf[1, rows, :] = y.astype(out_buf.dtype)

                    @when_last
                    def _():
                        for r in range(b * SQ // OUT_ROWS, (b + 1) * SQ // OUT_ROWS):
                            start_output(1, r, r % 2)

    jax.lax.fori_loop(0, STEPS - Q_AHEAD, lambda g, _: step(g, False), None)
    jax.lax.fori_loop(STEPS - Q_AHEAD, STEPS, lambda g, _: step(g, True), None)
    wait_filled(out_buf, out_sem)


def _pages(a):
    return a.reshape(-1, TILE_ROWS, NT, LANES).transpose(0, 2, 1, 3).reshape(-1, PAGE, LANES)


@jax.jit
def pallas_concat_heads__gqa_block_cached__mha_block_cached__near_ridge_kernel(
    A_x: jax.Array,
    A_k_cache: jax.Array,
    A_v_cache: jax.Array,
    A_wq: jax.Array,
    A_wo: jax.Array,
    B_x: jax.Array,
    B_k_cache: jax.Array,
    B_v_cache: jax.Array,
    B_wq: jax.Array,
    B_wo: jax.Array,
):
    assert A_x.shape == B_x.shape == (B, SQ, D)
    assert A_k_cache.shape == A_v_cache.shape == B_k_cache.shape == B_v_cache.shape == (B, H, SK, DH)
    dtype = A_x.dtype
    hbm = pl.BlockSpec(memory_space=pltpu.HBM)
    out = pl.pallas_call(
        _attention_kernel,
        out_shape=jax.ShapeDtypeStruct((M, 2 * D), dtype),
        in_specs=[hbm] * 10,
        out_specs=hbm,
        scratch_shapes=[
            pltpu.VMEM((SLOTS, B, SK, DH), dtype),
            pltpu.VMEM((SLOTS, B, SK, DH), dtype),
            pltpu.VMEM((STEPS // WQ_HEADS, D, WQ_COLS), dtype),
            pltpu.VMEM((SLOTS, NT * PAGE, LANES), dtype),
            pltpu.VMEM((DH, D), dtype),
            pltpu.VMEM((2, X_PAGES * PAGE, LANES), dtype),
            pltpu.VMEM((2, M, D), dtype),
            pltpu.VMEM((SLOTS, M, DH), dtype),
            pltpu.VMEM((M, DH), dtype),
            pltpu.VMEM((2, M, D), jnp.float32),
            pltpu.VMEM((2, M, D), dtype),
            pltpu.SemaphoreType.DMA((2 * SLOTS,)),
            pltpu.SemaphoreType.DMA((2 * SLOTS,)),
            pltpu.SemaphoreType.DMA((STEPS // WQ_HEADS,)),
            pltpu.SemaphoreType.DMA((SLOTS,)),
            pltpu.SemaphoreType.DMA(()),
            pltpu.SemaphoreType.DMA(()),
        ],
        compiler_params=pltpu.CompilerParams(vmem_limit_bytes=64 * 2**20),
        name="attn2",
    )(_pages(A_x), A_k_cache, A_v_cache, A_wq, _pages(A_wo),
      _pages(B_x), B_k_cache, B_v_cache, B_wq, _pages(B_wo))
    return out.reshape(B, SQ, 2 * D)
```

```python
import jax
import jax.numpy as jnp
import jax.experimental.pallas as pl
import jax.experimental.pallas.tpu as pltpu

B, SQ, D, H, SK, DH = 8, 96, 640, 32, 512, 128
M = B * SQ
STEPS = 2 * H
HALF = B // 2
LANES, TILE_ROWS = 128, 8
PAGE = 128
NT = D // LANES
X_PAGES = M * NT // PAGE
WQ_HEADS = 16
WQ_COLS = WQ_HEADS * DH
KV_PAGES = SK // PAGE
SLOTS = 4
SLOT_ROWS = NT * PAGE + 2 * B * SK
EARLY_ROWS = NT * PAGE + 2 * HALF * SK
Q_AHEAD = 3
AHEAD = (12, 20)
OUT_ROWS = 32
Q_SCALE = DH ** -0.5 * 1.4426950408889634


def _kv_pages(queue, by_halves):
    if by_halves:
        return [(a, HALF * p + 2 * b + queue, 2 * jj + j) for p in range(2) for jj in range(2)
                for a in range(2) for j in range(2) for b in range(2)]
    return [(a, 2 * b + queue, j) for j in range(KV_PAGES) for a in range(2) for b in range(HALF)]


def _block(i, size):
    return pl.ds(i * size if isinstance(i, int) else pl.multiple_of(i * size, size), size)


def _untile(pages):
    w = pages.astype(jnp.float32)
    tile = lambda r, c: w[(r * NT + c) * TILE_ROWS:(r * NT + c + 1) * TILE_ROWS]
    cols = [jnp.concatenate([tile(r, c) for r in range(128 // TILE_ROWS)], axis=0) for c in range(NT)]
    return jnp.concatenate(cols, axis=1).astype(pages.dtype)


def _attention_kernel(
        ax, ak, av, awq, awo, bx, bk, bv, bwq, bwo, out,
        ring, wq_buf, wo_buf, x_pages, x_buf, q_buf, o_buf, acc, out_buf,
        ring_sem, wq_sem, x_sem, out_sem):
    blocks = ((ak, av, awq, awo), (bk, bv, bwq, bwo))

    def start(src, dst, sem, queue):
        pltpu.make_async_copy(src, dst, sem).start(priority=queue)

    def wait_filled(buf, sem):
        pltpu.make_async_copy(buf, buf, sem).wait()

    def start_wq_page(wq, group, part, e, queue):
        rows = _block(part + e * WQ_HEADS, TILE_ROWS)
        start(wq.at[rows, _block(group & 1, WQ_COLS)], wq_buf.at[group, rows], wq_sem.at[group], queue)

    def plan(g):
        slot = g & (SLOTS - 1)
        gq = g + Q_AHEAD
        return dict(
            head=g & (H - 1), slot=slot, last=g == STEPS - 1,
            late_sem=jnp.where(g >= STEPS - Q_AHEAD, SLOTS + slot, slot),
            wq_group=((gq >> 4) + 1) & 3, wq_part=gq & (WQ_HEADS - 1),
            kv_from=((g >= 0) & (g < H), (g >= H) & (g < STEPS)),
            wq_from=((g >= 0) & (gq < WQ_HEADS), (gq >= WQ_HEADS) & (gq < H + WQ_HEADS)))

    def plans_after(g):
        return {i: plan(g + i) for i in range(min(AHEAD) // B, pl.cdiv(max(AHEAD), B) + 1)}

    def prefetch(work, sources=(0, 1), with_wq=True):
        for e in range(-1, 4):
            for queue, item in enumerate(work):
                if item is None:
                    continue
                p, part = item
                for i in sources:
                    k, v, wq, wo = blocks[i]
                    if e >= 0:
                        a, b, j = _kv_pages(queue, False)[4 * part + e]
                        late = b >= HALF
                        sem = p["late_sem"] if late else p["slot"]
                        if queue == 1 and i == 1:
                            _, b2, j2 = _kv_pages(queue, True)[4 * part + e]
                            sem2 = p["late_sem"] if b2 >= HALF else p["slot"]
                            if late != (b2 >= HALF):
                                sem = jnp.where(p["last"], sem2, sem)
                            b = b if b == b2 else jnp.where(p["last"], b2, b)
                            j = j if j == j2 else jnp.where(p["last"], j2, j)
                        pl.when(p["kv_from"][i])(lambda: start(
                            (k, v)[a].at[b, p["head"], _block(j, PAGE)],
                            ring.at[p["slot"], _block(NT + (2 * b + a) * KV_PAGES + j, PAGE)],
                            ring_sem.at[sem], queue))
                    elif part < NT and queue == 0:
                        pl.when(p["kv_from"][i])(lambda: start(
                            wo.at[p["head"] * NT + part], ring.at[p["slot"], _block(part, PAGE)],
                            ring_sem.at[p["slot"]], queue))
                    elif part < NT and with_wq:
                        pl.when(p["wq_from"][i])(lambda: start_wq_page(
                            wq, p["wq_group"], p["wq_part"], part, queue))

    def project_q(g, rows):
        w = wq_buf[g >> 4, :, _block(g & (WQ_HEADS - 1), DH)]
        q = jnp.dot(x_buf[g >> 5, rows, :], w, preferred_element_type=jnp.float32)
        q_buf[g & (SLOTS - 1), rows, :] = (q * Q_SCALE).astype(q_buf.dtype)

    def start_output(i, r, queue):
        rows = _block(r, OUT_ROWS)
        start(out_buf.at[i, rows], out.at[rows, _block(i, D)], out_sem, queue)

    def first_pages(i, _):
        for e in range(NT):
            start_wq_page(awq, 0, i, e, e % 2)
        for j in range(4):
            page = i + (X_PAGES // 2) * (j // 2)
            pl.when(i < X_PAGES // 2)(lambda: start(
                (ax, bx)[j % 2].at[page], x_pages.at[j % 2, _block(page, PAGE)], x_sem, (j + 1) % 2))
        for j in range(Q_AHEAD):
            pl.when(i < NT)(lambda: start_wq_page(awq, 1, j, i, (j + 1) % 2))

    def clear_acc(i, _):
        for j in range(2):
            acc[j, _block(i, 128), :] = jnp.zeros((128, D), acc.dtype)

    def untile_x(i, _):
        for j in range(2):
            x_buf[j, _block(i, 128), :] = _untile(x_pages[j, _block(i, NT * 128), :])

    def lead_in(g, _):
        plans = plans_after(g)
        for t in range(B):
            prefetch([(plans[(t + d) // B], (t + d) % B) for d in AHEAD], sources=(0,))
            stage = Q_AHEAD - (B - 1 - t) // 2
            if t % 2 == 1 and stage >= 0:
                @pl.when(g == -1)
                def _():
                    if stage == 0:
                        wait_filled(x_pages, x_sem)
                        wait_filled(wq_buf.at[0], wq_sem.at[0])
                        jax.lax.fori_loop(0, M // 128, untile_x, None)
                    else:
                        jax.lax.fori_loop(0, 2, lambda i, _: project_q(stage - 1, _block(i, M // 2)), None)

    jax.lax.fori_loop(0, WQ_HEADS, first_pages, None)
    jax.lax.fori_loop(0, M // 128, clear_acc, None)
    jax.lax.fori_loop(-pl.cdiv(max(AHEAD), B), 0, lead_in, None)

    def step(g, tail):
        slot, blk = g & (SLOTS - 1), g >> 5
        plans = plans_after(g)
        when_last = pl.when(g == STEPS - 1)
        if tail:
            wait_filled(ring.at[slot, pl.ds(0, EARLY_ROWS)], ring_sem.at[slot])
        else:
            group = (g + Q_AHEAD) >> 4
            pl.when(((g + Q_AHEAD) & (WQ_HEADS - 1)) == 0)(
                lambda: wait_filled(wq_buf.at[group], wq_sem.at[group]))

            @pl.when(g == H + B)
            def _():
                out_buf[0] = acc[0].astype(out_buf.dtype)

            wait_filled(ring.at[slot], ring_sem.at[slot])
        wo_buf[...] = _untile(ring[slot, pl.ds(0, NT * PAGE), :])
        cache = lambda a, b: ring[slot, pl.ds(NT * PAGE + (2 * b + a) * SK, SK), :]

        scores = {}
        for t in range(B + 2):
            if t < B:
                work = [(plans[(t + d) // B], (t + d) % B) if not tail or (t + d) // B < Q_AHEAD else None
                        for d in AHEAD]
                prefetch(work, sources=(1,) if tail else (0, 1), with_wq=not tail)
            if tail and t == 1:
                @when_last
                def _():
                    n = M // OUT_ROWS
                    for i in range(n):
                        start_output(0, (7 * i) % n, i % 2)
            if tail and t == HALF:
                wait_filled(ring.at[slot, pl.ds(EARLY_ROWS, SLOT_ROWS - EARLY_ROWS)], ring_sem.at[SLOTS + slot])
            if t < B:
                scores[t] = jax.lax.dot_general(
                    q_buf[slot, _block(t, SQ), :], cache(0, t), (((1,), (1,)), ((), ())),
                    preferred_element_type=jnp.float32)
                if not tail:
                    project_q(g + Q_AHEAD, _block(t, SQ))
            b = t - 1
            if 0 <= b < B:
                s = scores.pop(b)
                p = jnp.exp2(s - jnp.max(s, axis=-1, keepdims=True))
                total = jnp.sum(p, axis=-1, keepdims=True)
                o = jnp.dot(p.astype(ring.dtype), cache(1, b), preferred_element_type=jnp.float32)
                o_buf[_block(b, SQ), :] = (o * (1.0 / total)).astype(o_buf.dtype)
            b = t - 2
            if 0 <= b < B:
                rows = _block(b, SQ)
                y = acc[blk, rows, :] + jnp.dot(o_buf[rows, :], wo_buf[...], preferred_element_type=jnp.float32)
                acc[blk, rows, :] = y
                if tail:
                    out_buf[1, rows, :] = y.astype(out_buf.dtype)

                    @when_last
                    def _():
                        for r in range(b * SQ // OUT_ROWS, (b + 1) * SQ // OUT_ROWS):
                            start_output(1, r, r % 2)

    jax.lax.fori_loop(0, STEPS - Q_AHEAD, lambda g, _: step(g, False), None)
    jax.lax.fori_loop(STEPS - Q_AHEAD, STEPS, lambda g, _: step(g, True), None)
    wait_filled(out, out_sem)


def _pages(a):
    return a.reshape(-1, TILE_ROWS, NT, LANES).transpose(0, 2, 1, 3).reshape(-1, PAGE, LANES)


@jax.jit
def pallas_concat_heads__gqa_block_cached__mha_block_cached__near_ridge_kernel(
    A_x: jax.Array,
    A_k_cache: jax.Array,
    A_v_cache: jax.Array,
    A_wq: jax.Array,
    A_wo: jax.Array,
    B_x: jax.Array,
    B_k_cache: jax.Array,
    B_v_cache: jax.Array,
    B_wq: jax.Array,
    B_wo: jax.Array,
):
    assert A_x.shape == B_x.shape == (B, SQ, D)
    assert A_k_cache.shape == A_v_cache.shape == B_k_cache.shape == B_v_cache.shape == (B, H, SK, DH)
    dtype = A_x.dtype
    hbm = pl.BlockSpec(memory_space=pltpu.HBM)
    out = pl.pallas_call(
        _attention_kernel,
        out_shape=jax.ShapeDtypeStruct((M, 2 * D), dtype),
        in_specs=[hbm] * 10,
        out_specs=hbm,
        scratch_shapes=[
            pltpu.VMEM((SLOTS, SLOT_ROWS, LANES), dtype),
            pltpu.VMEM((STEPS // WQ_HEADS, D, WQ_COLS), dtype),
            pltpu.VMEM((DH, D), dtype),
            pltpu.VMEM((2, X_PAGES * PAGE, LANES), dtype),
            pltpu.VMEM((2, M, D), dtype),
            pltpu.VMEM((SLOTS, M, DH), dtype),
            pltpu.VMEM((M, DH), dtype),
            pltpu.VMEM((2, M, D), jnp.float32),
            pltpu.VMEM((2, M, D), dtype),
            pltpu.SemaphoreType.DMA((2 * SLOTS,)),
            pltpu.SemaphoreType.DMA((STEPS // WQ_HEADS,)),
            pltpu.SemaphoreType.DMA(()),
            pltpu.SemaphoreType.DMA(()),
        ],
        compiler_params=pltpu.CompilerParams(vmem_limit_bytes=64 * 2**20),
        name="attn2",
    )(_pages(A_x), A_k_cache, A_v_cache, A_wq, _pages(A_wo),
      _pages(B_x), B_k_cache, B_v_cache, B_wq, _pages(B_wo))
    return out.reshape(B, SQ, 2 * D)
```
